```python
import os as _os
_os.environ.setdefault('JAX_PLATFORMS', 'cpu')
import jax
import jax.numpy as jnp

def _softmax(x, axis=-1):
    return jax.nn.softmax(x, axis=axis)

def _gelu(x):
    return jax.nn.gelu(x, approximate=True)

def _silu(x):
    return jax.nn.silu(x)

def _sigmoid(x):
    return jax.nn.sigmoid(x)

def _layernorm(x, axis=-1, eps=1e-05):
    m = jnp.mean(x, axis=axis, keepdims=True)
    v = jnp.var(x, axis=axis, keepdims=True)
    return (x - m) / jnp.sqrt(v + eps)

def _scatter_add(tgt, idx, src, axis=0):
    return tgt.at[idx].add(src)

def _segment_sum(src, seg, n):
    return jax.ops.segment_sum(src, seg, n)

class _Rng:

    def __init__(self, key):
        self._k = key

    def _next(self):
        self._k, sub = jax.random.split(self._k)
        return sub

    def normal(self, shape):
        return jax.random.normal(self._next(), shape, dtype=jnp.bfloat16)

    def randint(self, lo, hi, shape):
        return jax.random.randint(self._next(), shape, lo, hi, dtype=jnp.int32)

    def uniform(self, shape, lo=0.0, hi=1.0):
        return jax.random.uniform(self._next(), shape, jnp.bfloat16, lo, hi)

    def permutation(self, n):
        return jax.random.permutation(self._next(), n)
kernel_name = 'standalone__conformer_conv_module__speech'

def setup_inputs():
    _rng = _Rng(jax.random.key(int.from_bytes(__import__("os").urandom(4), "little")))
    _w = lambda a: (lambda t: t.astype(jnp.bfloat16) if jnp.issubdtype(t.dtype, jnp.floating) else t)(jnp.asarray(a))
    B, T, D, K = (2, 16000, 256, 5)
    return {'x': _w((lambda *s: _rng.normal(s) * 0.2)(B, T, D)), 'w_pw1': _w((lambda *s: _rng.normal(s) * 0.2)(D, 2 * D)), 'dw': _w((lambda *s: _rng.normal(s) * 0.05)(K, D)), 'w_pw2': _w((lambda *s: _rng.normal(s) * 0.05)(D, D))}

def reference(x, w_pw1, dw, w_pw2):
    B, T, D = x.shape
    K = dw.shape[0]
    h = x @ w_pw1
    a, b = (h[..., :D].copy(), h[..., D:].copy())
    h = a * _sigmoid(b)
    pad = K // 2
    hp = jnp.pad(h, ((0, 0), (pad, pad), (0, 0)))
    out = jnp.zeros_like(h)
    for i in range(K):
        out = out + hp[:, i:i + T, :] * dw[i][None, None, :]
    return _silu(out) @ w_pw2
```

```python
import functools

import jax
import jax.numpy as jnp
from jax import lax
import jax.experimental.pallas as pl
import jax.experimental.pallas.tpu as pltpu

S = 160
RF = 22
RC = 26
FW = (2, 8)
LAG = 2
PAD = 8
NL = 2


def _kernel(x_hbm, w1_hbm, dw_hbm, w2_hbm, o_hbm,
            xbuf, obuf, g_ref, w1_ref, dw_ref, w2_ref, w1s_ref, dws_ref,
            fin_sem, in_sem, out_sem, tail_sem, w_sem, *, B, T, D, K):
    nsub = T // S
    k = (nsub - RF) // RC
    assert B == 2 and T % S == 0 and RF + k * RC == nsub and D == NL * 128
    NLOOP = 2 * k
    pad = K // 2

    def mo(v):
        return v if isinstance(v, int) else pl.multiple_of(v, 16)

    def icopy(q0, nq, sem):
        lo = mo(q0 * S)
        return pltpu.make_async_copy(x_hbm.at[pl.ds(lo, nq * S), :],
                                     xbuf.at[pl.ds(lo, nq * S), :], sem)

    def ocopy(q0, nq, sem):
        lo = mo(q0 * S)
        return pltpu.make_async_copy(obuf.at[pl.ds(lo, nq * S), :],
                                     o_hbm.at[pl.ds(lo, nq * S), :], sem)

    fb = [0] + list(FW) + [RF + LAG]
    fin = [icopy(fb[i], fb[i + 1] - fb[i], fin_sem.at[i]) for i in range(len(fb) - 1)]

    def lin(J):
        return icopy(RF + J * RC + LAG, RC, in_sem.at[J])

    lin_last = icopy(RF + NLOOP * RC + LAG, RF - LAG, in_sem.at[NLOOP])

    def lout(J):
        return ocopy(RF + J * RC, RC, out_sem.at[1 + J])

    fout = ocopy(0, RF, out_sem.at[0])

    wcopies = [pltpu.make_async_copy(w1_hbm, w1_ref, w_sem.at[0]),
               pltpu.make_async_copy(dw_hbm, dw_ref, w_sem.at[1]),
               pltpu.make_async_copy(w2_hbm, w2_ref, w_sem.at[2])]
    wcopies[0].start()
    fin[0].start()
    wcopies[1].start()
    wcopies[2].start()
    fin[1].start()

    zeros = jnp.zeros((PAD, 128), jnp.float32)
    for l in range(NL):
        g_ref[l, 0:PAD, :] = zeros
    wcopies[0].wait()
    for c in fin[2:]:
        c.start()
    lin(0).start()
    w1s_ref[...] = (w1_ref[...].astype(jnp.float32) * 0.5).astype(jnp.bfloat16)

    def stage_a(q, slot, R, keep):
        xx = xbuf[pl.ds(mo(q * S), S), :]
        gb = PAD + slot * S
        h = jnp.dot(xx, w1s_ref[...], preferred_element_type=jnp.float32)
        for l in range(NL):
            a = h[:, l * 128:(l + 1) * 128]
            b = h[:, D + l * 128:D + (l + 1) * 128]
            g = a * jnp.tanh(b) + a
            g_ref[l, gb:gb + S, :] = g
            if slot == 0 and keep is not None:
                head = g[0:PAD]
                g_ref[l, PAD + R * S:PAD + R * S + PAD, :] = (
                    head if keep is True else jnp.where(keep, head, 0.0))
            if slot == R - 1 and keep is not None:
                tail = g[S - PAD:S]
                g_ref[l, 0:PAD, :] = tail if keep is True else jnp.where(keep, tail, 0.0)

    def stage_b(q, slot):
        gb = PAD + slot * S
        ys = []
        for l in range(NL):
            acc = None
            for i in range(K):
                lo = gb + i - pad
                term = g_ref[l, lo:lo + S, :] * dws_ref[i:i + 1, l * 128:(l + 1) * 128]
                acc = term if acc is None else acc + term
            ys.append((acc * jnp.tanh(acc) + acc).astype(jnp.bfloat16))
        y = jnp.concatenate(ys, axis=1)
        obuf[pl.ds(mo(q * S), S), :] = jnp.dot(
            y, w2_ref[...], preferred_element_type=jnp.float32).astype(obuf.dtype)

    fin[0].wait()
    for q in range(LAG):
        stage_a(q, q, RF, None)
    wcopies[1].wait()
    wcopies[2].wait()
    dws_ref[0:K, :] = dw_ref[...].astype(jnp.float32) * 0.5

    for s in range(RF):
        qa = s + LAG
        if qa in FW:
            fin[1 + FW.index(qa)].wait()
        stage_a(qa, qa % RF, RF, True)
        stage_b(s, s)

    def body(J, c):
        lin(J).wait()

        @pl.when(J + 1 < NLOOP)
        def _():
            lin(J + 1).start()

        @pl.when(J + 1 == NLOOP)
        def _():
            lin_last.start()

        @pl.when(J == 0)
        def _():
            fout.start()

        @pl.when(J >= 1)
        def _():
            lout(J - 1).start()

        keep = J != (k - 1)
        q0 = RF + J * RC
        for s in range(RC):
            stage_a(q0 + s + LAG, (s + LAG) % RC, RC, keep)
            stage_b(q0 + s, s)
        return c

    lax.fori_loop(0, NLOOP, body, 0)

    lin_last.wait()
    lout(NLOOP - 1).start()
    q0 = RF + NLOOP * RC
    for l in range(NL):
        g_ref[l, PAD + RF * S:PAD + RF * S + PAD, :] = zeros
    tails = []
    for s in range(RF):
        if s + LAG < RF:
            stage_a(q0 + s + LAG, s + LAG, RF, None)
        stage_b(q0 + s, s)
        tc = ocopy(q0 + s, 1, tail_sem.at[s])
        tc.start()
        tails.append(tc)
    fout.wait()
    for J in range(NLOOP):
        lout(J).wait()
    for tc in tails:
        tc.wait()


@jax.jit
def pallas_standalone__conformer_conv_module__speech_kernel(
    x: jax.Array,
    w_pw1: jax.Array,
    dw: jax.Array,
    w_pw2: jax.Array,
):
    B, T, D = x.shape
    K = dw.shape[0]
    NLOOP = 2 * ((T // S - RF) // RC)
    out = pl.pallas_call(
        functools.partial(_kernel, B=B, T=T, D=D, K=K),
        in_specs=[pl.BlockSpec(memory_space=pl.ANY)] * 4,
        out_specs=pl.BlockSpec(memory_space=pl.ANY),
        out_shape=jax.ShapeDtypeStruct((B * T, D), x.dtype),
        scratch_shapes=[
            pltpu.VMEM((B * T, D), jnp.bfloat16),
            pltpu.VMEM((B * T, D), jnp.bfloat16),
            pltpu.VMEM((NL, max(RF, RC) * S + 2 * PAD, 128), jnp.float32),
            pltpu.VMEM((D, 2 * D), jnp.bfloat16),
            pltpu.VMEM((K, D), jnp.bfloat16),
            pltpu.VMEM((D, D), jnp.bfloat16),
            pltpu.VMEM((D, 2 * D), jnp.bfloat16),
            pltpu.VMEM((8, D), jnp.float32),
            pltpu.SemaphoreType.DMA((len(FW) + 1,)),
            pltpu.SemaphoreType.DMA((NLOOP + 1,)),
            pltpu.SemaphoreType.DMA((NLOOP + 1,)),
            pltpu.SemaphoreType.DMA((RF,)),
            pltpu.SemaphoreType.DMA((3,)),
        ],
        compiler_params=pltpu.CompilerParams(vmem_limit_bytes=110 * 1024 * 1024),
    )(x.reshape(B * T, D), w_pw1, dw, w_pw2)
    return out.reshape(B, T, D)
```
